```python
import os as _os
_os.environ.setdefault("JAX_PLATFORMS", "cpu")
import jax
import jax.numpy as jnp

def _softmax(x, axis=-1):
    return jax.nn.softmax(x, axis=axis)
def _gelu(x):
    return jax.nn.gelu(x, approximate=True)
def _silu(x):
    return jax.nn.silu(x)
def _sigmoid(x):
    return jax.nn.sigmoid(x)
def _layernorm(x, axis=-1, eps=1e-5):
    m = jnp.mean(x, axis=axis, keepdims=True)
    v = jnp.var(x, axis=axis, keepdims=True)
    return (x - m) / jnp.sqrt(v + eps)
def _scatter_add(tgt, idx, src, axis=0):
    return tgt.at[idx].add(src)
def _segment_sum(src, seg, n):
    return jax.ops.segment_sum(src, seg, n)
class _Rng:
    def __init__(self, key):
        self._k = key
    def _next(self):
        self._k, sub = jax.random.split(self._k)
        return sub
    def normal(self, shape):
        return jax.random.normal(self._next(), shape, dtype=jnp.bfloat16)
    def randint(self, lo, hi, shape):
        return jax.random.randint(self._next(), shape, lo, hi, dtype=jnp.int32)
    def uniform(self, shape, lo=0.0, hi=1.0):
        return jax.random.uniform(self._next(), shape, jnp.bfloat16, lo, hi)
    def permutation(self, n):
        return jax.random.permutation(self._next(), n)


kernel_name = 'standalone__seq2seq_rnn_t_joint__speech'

def setup_inputs():
    _rng = _Rng(jax.random.key(int.from_bytes(__import__("os").urandom(4), "little")))
    _w = (lambda a: (lambda t: t.astype(jnp.bfloat16) if jnp.issubdtype(t.dtype, jnp.floating) else t)(jnp.asarray(a)))
    B, T, D, K = 2, 16000, 256, 31
    U = 8
    sc = (1.0 / (K * D)) ** 0.5
    sd = (1.0 / D) ** 0.5
    return {
        "x": _w((lambda *s: _rng.normal(s) * 0.2)(B, T, D) * 0.5),
        "w1": _w((lambda *s: _rng.normal(s) * 1.6)(K, D, D) * sc),
        "w2": _w((lambda *s: _rng.normal(s) * 1.6)(K, D, D) * sc),
        "g": _w((lambda *s: _rng.normal(s) * 1.6)(B, U, D) * 0.5),
        "w_f": _w((lambda *s: _rng.normal(s) * 1.6)(D, D) * sd),
        "w_g": _w((lambda *s: _rng.normal(s) * 1.6)(D, D) * sd),
        "w_o": _w((lambda *s: _rng.normal(s) * 1.6)(D, D) * sd),
    }

def reference(x, w1, w2, g, w_f, w_g, w_o):
    B, T, D = x.shape
    K = w1.shape[0]
    pad = K // 2
    xp = jnp.pad(x, ((0,0),(pad,pad),(0,0)))
    h = jnp.zeros_like(x)
    for i in range(K):
        h = h + jnp.einsum("btc,cd->btd", xp[:, i:i+T, :], w1[i])
    h = _gelu(h)[:, ::2, :]
    T1 = h.shape[1]
    hp = jnp.pad(h, ((0,0),(pad,pad),(0,0)))
    f = jnp.zeros_like(h)
    for i in range(K):
        f = f + jnp.einsum("btc,cd->btd", hp[:, i:i+T1, :], w2[i])
    f = _gelu(f)[:, ::2, :]
    fe = jnp.einsum("btd,de->bte", f, w_f)
    ge = jnp.einsum("bud,de->bue", g, w_g)
    j = jnp.tanh(fe[:, :, None, :] + ge[:, None, :, :])
    return jnp.einsum("btud,dv->btuv", j, w_o)
```

```python
import jax
import jax.numpy as jnp
import jax.experimental.pallas as pl
import jax.experimental.pallas.tpu as pltpu

F32, BF16 = jnp.float32, jnp.bfloat16
NSEG = 16
R = 16
NP = 81


def _data_tf(d):
    if len(d) == 1:
        return d
    h = (len(d) + 1) // 4
    lo, mid, hi = d[:2 * h - 1], d[h:3 * h - 1], d[2 * h:]
    return (_data_tf([a - b for a, b in zip(lo, mid)]) + _data_tf(mid)
            + _data_tf([a - b for a, b in zip(hi, mid)]))


def _add(a, b):
    return b if a is None else a if b is None else a + b


def _weight_tf(g):
    if len(g) == 1:
        return g
    h = len(g) // 2
    return (_weight_tf(g[:h]) + _weight_tf([_add(a, b) for a, b in zip(g[:h], g[h:])])
            + _weight_tf(g[h:]))


def _out_tf(m):
    if len(m) == 1:
        return [m[0]()]
    h = len(m) // 3
    a, b, c = _out_tf(m[:h]), _out_tf(m[h:2 * h]), _out_tf(m[2 * h:])
    return [x + y for x, y in zip(a, b)] + [x + y for x, y in zip(b, c)]


def _u(v):
    return pltpu.pack_elementwise([v[:8], v[8:]], packed_dtype=BF16).astype(jnp.uint32)


def _half(w, ph):
    return pltpu.bitcast(w << 16 if ph == 0 else w & jnp.uint32(0xFFFF0000), F32)


def _eo(v):
    w = pltpu.bitcast(v, jnp.uint32)
    return jnp.concatenate([_half(w, 0), _half(w, 1)], axis=0)


def _b(v):
    return pltpu.bitcast(v, BF16)


def _gelu(x):
    return jax.nn.gelu(x, approximate=True)


@jax.jit
def pallas_standalone__seq2seq_rnn_t_joint__speech_kernel(
    x: jax.Array, w1: jax.Array, w2: jax.Array, g: jax.Array,
    w_f: jax.Array, w_g: jax.Array, w_o: jax.Array,
):
    B, T, D = x.shape
    U = g.shape[1]
    assert (B, T, D, U, w1.shape[0]) == (2, 16000, 256, 8, 31)
    SPB = NSEG // B
    L0 = T // SPB
    L1, L2 = L0 // 2, L0 // 4
    NB1, NT1 = 9, 7
    NB2, NT2 = 8, 4
    XP = 2048
    HP = 2 * (R * NB2 * NT2 + R)
    CH = 2 * R * NB1
    TB = 10
    NJ = L2 // TB

    def kernel(x_hbm, w1_hbm, w2_hbm, g_ref, wf_ref, wg_ref, wo_ref, o_hbm,
               xa, xb, sa, sb, wraw, wt, dd_, pp, h, f, fe, wfs, wos, ob0, ob1,
               xsem, wsem, osem):
        xs = (xa, xb)

        def x_copies(c, si=None):
            lo = 0 if c == 0 else c * CH + 2 * R
            hi = min((c + 1) * CH + 2 * R, XP)
            out = []
            for s in range(NSEG):
                base = (s % SPB) * L0 - R
                a, b = max(lo, -base), min(hi, T - base)
                for k in range(2):
                    out.append(pltpu.make_async_copy(
                        x_hbm.at[s // SPB, pl.ds(base + a, b - a), pl.ds(k * 128, 128)],
                        xs[k].bitcast(BF16).at[pl.ds(s * XP + a, b - a), :], xsem.at[c if si is None else si]))
            return out

        cw1 = pltpu.make_async_copy(w1_hbm, wraw, wsem.at[0])
        cw2 = pltpu.make_async_copy(w2_hbm, wraw, wsem.at[1])
        cw1.start()
        for c in range(1):
            for cp in x_copies(c):
                cp.start()
        for k in range(2):
            for b in range(B):
                xs[k][pl.ds(b * SPB * XP // 2, R // 2), :] = jnp.zeros((R // 2, 128), jnp.uint32)
                xs[k][pl.ds((((b + 1) * SPB - 1) * XP + R + L0) // 2, (XP - R - L0) // 2), :] = (
                    jnp.zeros(((XP - R - L0) // 2, 128), jnp.uint32))

        def weight_stage():
            def body(i, _):
                r = pl.ds(pl.multiple_of(i * 16, 16), 16)
                for ph in range(2):
                    r2 = pl.ds(pl.multiple_of(ph * D // 2 + i * 8, 8), 8)
                    for k in range(2):
                        ln = pl.ds(k * 128, 128)
                        taps = [None if 2 * j + ph == 0 else
                                _eo(wraw[2 * j + ph - 1, r, ln]) for j in range(R)]
                        for p, v in enumerate(_weight_tf(taps)):
                            wt[p, r2, ln] = jnp.zeros((8, 128), jnp.uint32) if v is None else _u(v)
            jax.lax.fori_loop(0, D // 16, body, None)

        def tf(d, b, loads):
            rows = pl.ds(pl.multiple_of(b * 8, 8), 8)
            pts = (((0, 1), (1, -1)), ((1, 1),), ((2, 1), (1, -1)))
            for gi in range(9):
                for col, ld in loads:
                    dd = []
                    for e in range(7):
                        acc = None
                        for qa, sa_ in pts[gi // 3]:
                            inner = None
                            for qb, _ in pts[gi % 3]:
                                v = ld(8 * qa + 4 * qb + e)
                                inner = v if inner is None else inner - v
                            acc = inner if acc is None else acc - inner
                        dd.append(acc)
                    for p, v in enumerate(_data_tf(dd)):
                        d[gi * 9 + p, rows, pl.ds(col, 128)] = _u(v)
                if gi not in (2, 5):
                    yield

        def a1(d, blk, b):
            loads = []
            for k in range(2):
                xw = (sa, sb)[k]
                for sg in range(NSEG):
                    xw[pl.ds((sg // 2 + sg % 2 * 8) * 33, 32), :] = xs[k][pl.ds(pl.multiple_of(sg * XP // 2 + blk * R, 8), 32), :]
                for ph in range(2):
                    loads.append((ph * D + k * 128, lambda q, xw=xw, ph=ph: _half(
                        xw[pl.ds(q, NSEG, stride=33), :], ph)))
            return tf(d, b, loads)

        def a2(d, blk, b):
            return tf(d, b, [(ph * D + k * 128, lambda q, k=k, ph=ph: _eo(
                h[2 * (blk * R + q) + ph, :, pl.ds(k * 128, 128)]))
                for ph in range(2) for k in range(2)])

        def make_c(dst, off):
            def c(pb, blk, b):
                rows = pl.ds(pl.multiple_of(b * NSEG, NSEG), NSEG)
                for k in range(2):
                    ln = pl.ds(k * 128, 128)
                    ys = _out_tf([(lambda p=p: pb[p, rows, ln]) for p in range(NP)])
                    for q, y in enumerate(ys):
                        dst[off + blk * R + q, :, ln] = _gelu(y).astype(BF16)
                    yield
            return c

        def conv(nb, nt, stage_a, stage_c, pre, last):
            m = pl.ds(0, nb * NSEG)
            q = NP // nb

            def mm(t, p, z=0):
                pp[t % 2 + z, p, m, :] = jnp.dot(_b(dd_[t % 2 + z, p, pl.ds(0, nb * 8), :]), _b(wt[p]),
                                             preferred_element_type=F32)

            def tile(t, da, db, dc):
                if da:
                    pre(t + 1)

                def body(i, _):
                    gs = []
                    if da:
                        gs.append(stage_a(dd_.at[(t + 1) % 2], (t + 1) * nb + i, i))
                    if dc:
                        gs.append(stage_c(pp.at[(t - 1) % 2], (t - 1) * nb + i, i))
                    for r in range(q):
                        if db:
                            mm(t, i * q + r, i >> 8)
                        for gen in gs:
                            next(gen, None)
                jax.lax.fori_loop(0, nb, body, None)
                if db:
                    for p in range(q * nb, NP):
                        mm(t, p)

            tile(-1, 1, 0, 0)
            tile(0, 1, 1, 0)
            jax.lax.fori_loop(1, last, lambda t, _: tile(t, 1, 1, 1), None)
            for t in range(last, nt - 1):
                tile(t, 1, 1, 1)
            tile(nt - 1, 0, 1, 1)
            tile(nt, 0, 0, 1)

        def wait_x(c):
            for cp in (x_copies(c) if isinstance(c, int) else x_copies(1, c)):
                cp.wait()
            if isinstance(c, int):
                if c == 1:
                    for cp in x_copies(2):
                        cp.start()
                if c == NT1 - 1:
                    cw2.start()
            else:
                for n in range(3, NT1):
                    @pl.when(c + 1 == n)
                    def _():
                        for cp in x_copies(n):
                            cp.start()

        cw1.wait()
        weight_stage()
        for c in range(1, 2):
            for cp in x_copies(c):
                cp.start()
        conv(NB1, NT1, a1, make_c(h, R), wait_x, NT1 - 2)
        cw2.wait()
        weight_stage()

        seg = jax.lax.broadcasted_iota(jnp.int32, (NSEG, D), 0) % SPB
        for q in range(R):
            v = pltpu.roll(h[L1 + q].astype(F32), 1, 0)
            h[q] = jnp.where(seg == 0, 0.0, v).astype(BF16)
            v = pltpu.roll(h[R + q].astype(F32), NSEG - 1, 0)
            h[R + L1 + q] = jnp.where(seg == SPB - 1, 0.0, v).astype(BF16)
        h[pl.ds(2 * R + L1, HP - 2 * R - L1)] = jnp.zeros((HP - 2 * R - L1, NSEG, D), BF16)

        conv(NB2, NT2, a2, make_c(f, 0), lambda t: None, NT2 - 1)

        wfs[...] = wf_ref[...]
        wos[...] = wo_ref[...]
        ge = jnp.dot(g_ref[...], wg_ref[...], preferred_element_type=F32)
        fe[...] = jnp.dot(f[pl.ds(0, L2)].reshape(L2 * NSEG, D), wfs[...],
                          preferred_element_type=F32).reshape(L2, NSEG, D)
        ges = (ge[:U], ge[U:])

        def ocopy(i, ob, k):
            rows = pl.ds(pl.multiple_of(i * TB * U, 16), TB * U)
            return pltpu.make_async_copy(ob, o_hbm.at[:, rows, :], osem.at[k])

        def jbody(i2, _):
            for k, ob in enumerate((ob0, ob1)):
                i = 2 * i2 + k

                @pl.when(i2 > 0)
                def _():
                    ocopy(i - 2, ob, k).wait()

                j = jnp.concatenate(
                    [jnp.tanh(fe[i * TB + t, pl.ds(s, 1), :] + ges[s // SPB])
                     for s in range(NSEG) for t in range(TB)], axis=0).astype(BF16)
                y = jnp.dot(j, wos[...], preferred_element_type=F32)
                ob[...] = y.astype(BF16).reshape(NSEG, TB * U, D)
                ocopy(i, ob, k).start()
        jax.lax.fori_loop(0, NJ // 2, jbody, None)
        ocopy(NJ - 2, ob0, 0).wait()
        ocopy(NJ - 1, ob1, 1).wait()

    hbm = pl.BlockSpec(memory_space=pl.ANY)
    vm = pl.BlockSpec(memory_space=pltpu.VMEM)
    V = pltpu.VMEM
    M = NB1 * NSEG
    out = pl.pallas_call(
        kernel,
        in_specs=[hbm, hbm, hbm, vm, vm, vm, vm],
        out_specs=hbm,
        out_shape=jax.ShapeDtypeStruct((NSEG, L2 * U, D), BF16),
        scratch_shapes=[
            V((NSEG * XP // 2, 128), jnp.uint32), V((NSEG * XP // 2, 128), jnp.uint32),
            V((NSEG * 33, 128), jnp.uint32), V((NSEG * 33, 128), jnp.uint32),
            V((31, D, D), BF16), V((NP, D, D), jnp.uint32),
            V((2, NP, M // 2, 2 * D), jnp.uint32),
            V((2, NP, M, D), F32),
            V((HP, NSEG, D), BF16), V((R * NB2 * NT2, NSEG, D), BF16),
            V((L2, NSEG, D), F32), V((D, D), BF16), V((D, D), BF16),
            V((NSEG, TB * U, D), BF16), V((NSEG, TB * U, D), BF16),
            pltpu.SemaphoreType.DMA((NT1,)), pltpu.SemaphoreType.DMA((2,)),
            pltpu.SemaphoreType.DMA((2,)),
        ],
        compiler_params=pltpu.CompilerParams(vmem_limit_bytes=125 * 1024 * 1024),
    )(x, w1, w2, g.reshape(B * U, D), w_f, w_g, w_o)
    return out.reshape(B, T // 4, U, D)
```
